```python
import os as _os
_os.environ.setdefault("JAX_PLATFORMS", "cpu")
import jax
import jax.numpy as jnp

def _softmax(x, axis=-1):
    return jax.nn.softmax(x, axis=axis)
def _gelu(x):
    return jax.nn.gelu(x, approximate=True)
def _silu(x):
    return jax.nn.silu(x)
def _sigmoid(x):
    return jax.nn.sigmoid(x)
def _layernorm(x, axis=-1, eps=1e-5):
    m = jnp.mean(x, axis=axis, keepdims=True)
    v = jnp.var(x, axis=axis, keepdims=True)
    return (x - m) / jnp.sqrt(v + eps)
def _scatter_add(tgt, idx, src, axis=0):
    return tgt.at[idx].add(src)
def _segment_sum(src, seg, n):
    return jax.ops.segment_sum(src, seg, n)
class _Rng:
    def __init__(self, key):
        self._k = key
    def _next(self):
        self._k, sub = jax.random.split(self._k)
        return sub
    def normal(self, shape):
        return jax.random.normal(self._next(), shape, dtype=jnp.bfloat16)
    def randint(self, lo, hi, shape):
        return jax.random.randint(self._next(), shape, lo, hi, dtype=jnp.int32)
    def uniform(self, shape, lo=0.0, hi=1.0):
        return jax.random.uniform(self._next(), shape, jnp.bfloat16, lo, hi)
    def permutation(self, n):
        return jax.random.permutation(self._next(), n)


kernel_name = 'concat_heads__mha_block_cached__gqa_block_cached__near_ridge'

def setup_inputs():
    _rng = _Rng(jax.random.key(int.from_bytes(__import__("os").urandom(4), "little")))
    _w = (lambda a: (lambda t: t.astype(jnp.bfloat16) if jnp.issubdtype(t.dtype, jnp.floating) else t)(jnp.asarray(a)))
    def _A_setup():
        B, Sq, D = 8, 128, 512
        H, Sk, Dh = 32, 1024, 128
        return {
            "x": _w((lambda *s: _rng.normal(s) * 0.8)(B, Sq, D)),
            "k_cache": _w((lambda *s: _rng.normal(s) * 0.8)(B, H, Sk, Dh)),
            "v_cache": _w((lambda *s: _rng.normal(s) * 0.05)(B, H, Sk, Dh)),
            "wq": _w((lambda *s: _rng.normal(s) * 0.8)(D, H * Dh) * (D ** -0.5)),
            "wo": _w((lambda *s: _rng.normal(s) * 0.05)(H * Dh, D) * ((H * Dh) ** -0.5)),
        }
    _A_in = _A_setup()

    def _B_setup():
        B, Sq, D = 8, 128, 512
        Hq, Hkv, Sk, Dh = 32, 32, 1024, 128
        assert Hq % Hkv == 0, (Hq, Hkv)
        return {
            "x": _w((lambda *s: _rng.normal(s) * 0.8)(B, Sq, D)),
            "k_cache": _w((lambda *s: _rng.normal(s) * 0.8)(B, Hkv, Sk, Dh)),
            "v_cache": _w((lambda *s: _rng.normal(s) * 0.05)(B, Hkv, Sk, Dh)),
            "wq": _w((lambda *s: _rng.normal(s) * 0.8)(D, Hq * Dh) * (D ** -0.5)),
            "wo": _w((lambda *s: _rng.normal(s) * 0.05)(Hq * Dh, D) * ((Hq * Dh) ** -0.5)),
        }
    _B_in = _B_setup()

    return {
        "A_x": _A_in["x"],
        "A_k_cache": _A_in["k_cache"],
        "A_v_cache": _A_in["v_cache"],
        "A_wq": _A_in["wq"],
        "A_wo": _A_in["wo"],
        "B_x": _B_in["x"],
        "B_k_cache": _B_in["k_cache"],
        "B_v_cache": _B_in["v_cache"],
        "B_wq": _B_in["wq"],
        "B_wo": _B_in["wo"],
    }

def reference(A_x, A_k_cache, A_v_cache, A_wq, A_wo, B_x, B_k_cache, B_v_cache, B_wq, B_wo):
    def _A_ref(x, k_cache, v_cache, wq, wo):
        B, Sq, D = x.shape
        H, Dh = 32, 128
        q = (lambda x, *d: x.transpose(*d))((x @ wq).reshape(B, Sq, H, Dh), 0, 2, 1, 3)
        scores = jnp.einsum("bhqd,bhkd->bhqk", q, k_cache) * (Dh ** -0.5)
        p = _softmax(scores, axis=-1)
        o = jnp.einsum("bhqk,bhkd->bhqd", p, v_cache)
        return (lambda x, *d: x.transpose(*d))(o, 0, 2, 1, 3).reshape(B, Sq, H * Dh) @ wo

    def _B_ref(x, k_cache, v_cache, wq, wo):
        B, Sq, D = x.shape
        Hq, Dh = 32, 128
        Hkv = k_cache.shape[1]
        rep = Hq // Hkv
        q = (lambda x, *d: x.transpose(*d))((x @ wq).reshape(B, Sq, Hq, Dh), 0, 2, 1, 3)
        k = jnp.repeat(k_cache, rep, axis=1)
        v = jnp.repeat(v_cache, rep, axis=1)
        scores = jnp.einsum("bhqd,bhkd->bhqk", q, k) * (Dh ** -0.5)
        p = _softmax(scores, axis=-1)
        o = jnp.einsum("bhqk,bhkd->bhqd", p, v)
        return (lambda x, *d: x.transpose(*d))(o, 0, 2, 1, 3).reshape(B, Sq, Hq * Dh) @ wo

    a = _A_ref(A_x, A_k_cache, A_v_cache, A_wq, A_wo)
    b = _B_ref(B_x, B_k_cache, B_v_cache, B_wq, B_wo)
    return jnp.concatenate([a, b], axis=-1)
```

```python
import functools

import jax
import jax.numpy as jnp
import jax.experimental.pallas as pl
import jax.experimental.pallas.tpu as pltpu

HG = 2
NBUF = 2
LOG2E = 1.4426950408889634


def _kernel(ax, ak, av, awq, awo, bx, bk, bv, bwq, bwo, out_ref, acc_ref, *, hg, dh, d):
    g = pl.program_id(0)
    b = pl.program_id(1)
    c = (dh ** -0.5) * LOG2E

    def branch(x_ref, k_ref, v_ref, wq_ref, wo_ref):
        q = jnp.dot(x_ref[b], wq_ref[...], preferred_element_type=jnp.float32).astype(jnp.bfloat16)
        os_ = []
        for h in range(hg):
            s = jax.lax.dot_general(q[:, h * dh:(h + 1) * dh], k_ref[h], (((1,), (1,)), ((), ())),
                                    preferred_element_type=jnp.float32)
            m = jnp.max(s, axis=-1, keepdims=True)
            p = jnp.exp2((s - m) * c)
            l = jnp.sum(p, axis=-1, keepdims=True)
            o = jnp.dot(p.astype(jnp.bfloat16), v_ref[h], preferred_element_type=jnp.float32)
            os_.append((o * (1.0 / l)).astype(jnp.bfloat16))
        o = jnp.concatenate(os_, axis=-1) if hg > 1 else os_[0]
        return jnp.dot(o, wo_ref[...], preferred_element_type=jnp.float32)

    r = jnp.concatenate([branch(ax, ak, av, awq, awo), branch(bx, bk, bv, bwq, bwo)], axis=-1)

    @pl.when(g == 0)
    def _():
        acc_ref[b] = r

    @pl.when(g > 0)
    def _():
        acc_ref[b] += r

    @pl.when(g == pl.num_programs(0) - 1)
    def _():
        out_ref[...] = acc_ref[b].astype(out_ref.dtype)


@jax.jit
def pallas_concat_heads__mha_block_cached__gqa_block_cached__near_ridge_kernel(
    A_x, A_k_cache, A_v_cache, A_wq, A_wo, B_x, B_k_cache, B_v_cache, B_wq, B_wo,
):
    B, Sq, D = A_x.shape
    _, H, Sk, Dh = A_k_cache.shape
    hg = HG
    G = H // hg
    xs = pl.BlockSpec((B, Sq, D), lambda g, b: (0, 0, 0))
    kv = pl.BlockSpec((None, hg, Sk, Dh), lambda g, b: (b, g, 0, 0))
    wq = pl.BlockSpec((D, hg * Dh), lambda g, b: (0, g))
    wo = pl.BlockSpec((hg * Dh, D), lambda g, b: (g, 0))
    return pl.pallas_call(
        functools.partial(_kernel, hg=hg, dh=Dh, d=D),
        grid=(G, B),
        in_specs=[xs, kv, kv, wq, wo] * 2,
        out_specs=pl.BlockSpec((None, Sq, 2 * D), lambda g, b: (jnp.where(g == G - 1, b, 0), 0, 0)),
        out_shape=jax.ShapeDtypeStruct((B, Sq, 2 * D), A_x.dtype),
        scratch_shapes=[pltpu.VMEM((B, Sq, 2 * D), jnp.float32)],
        compiler_params=pltpu.CompilerParams(
            dimension_semantics=("arbitrary", "arbitrary"), vmem_limit_bytes=100 * 1024 * 1024),
    )(A_x, A_k_cache, A_v_cache, A_wq, A_wo, B_x, B_k_cache, B_v_cache, B_wq, B_wo)
```

```python
import functools

import jax
import jax.numpy as jnp
import jax.experimental.pallas as pl
import jax.experimental.pallas.tpu as pltpu

HG = 2
NBUF = 6
LOG2E = 1.4426950408889634


def _kernel(ax, ak, av, awq, awo, bx, bk, bv, bwq, bwo, out_hbm,
            x_buf, kv_buf, wq_buf, wo_buf, acc_ref, out_buf,
            x_sem, kv_sem, w_sem, o_sem, *, hg, nbuf):
    nb, sq, d = ax.shape
    nh, dh = ak.shape[1], ak.shape[3]
    ng = nh // hg
    nsteps = ng * nb
    w = hg * dh
    c = (dh ** -0.5) * LOG2E
    kv_src = (ak, av, bk, bv)

    def x_cp(j):
        return pltpu.make_async_copy((ax, bx)[j], x_buf.at[j], x_sem.at[j])

    def kv_cp(i, j):
        slot = i % nbuf
        return pltpu.make_async_copy(
            kv_src[j].at[i % nb, pl.ds((i // nb) * hg, hg)], kv_buf.at[slot, j], kv_sem.at[slot, j])

    def w_cps(g):
        slot = g % 2
        off = g * w if isinstance(g, int) else pl.multiple_of(g * w, w)
        return [
            pltpu.make_async_copy(awq.at[:, pl.ds(off, w)], wq_buf.at[slot, 0], w_sem.at[slot, 0]),
            pltpu.make_async_copy(bwq.at[:, pl.ds(off, w)], wq_buf.at[slot, 1], w_sem.at[slot, 1]),
            pltpu.make_async_copy(awo.at[pl.ds(off, w), :], wo_buf.at[slot, 0], w_sem.at[slot, 2]),
            pltpu.make_async_copy(bwo.at[pl.ds(off, w), :], wo_buf.at[slot, 1], w_sem.at[slot, 3]),
        ]

    def o_cp(b):
        return pltpu.make_async_copy(out_buf.at[b], out_hbm.at[b], o_sem.at[b])

    x_cp(0).start()
    x_cp(1).start()
    for cp in w_cps(0):
        cp.start()
    for i in range(nbuf - 1):
        for j in range(4):
            kv_cp(i, j).start()
    x_cp(0).wait()
    x_cp(1).wait()

    def step(i, _):
        g = i // nb
        b = i % nb
        slot = i % nbuf
        ws = g % 2

        @pl.when(i + nbuf - 1 < nsteps)
        def _():
            for j in range(4):
                kv_cp(i + nbuf - 1, j).start()

        @pl.when(b == 0)
        def _():
            for cp in w_cps(g):
                cp.wait()

            @pl.when(g + 1 < ng)
            def _():
                for cp in w_cps(g + 1):
                    cp.start()

        for j in range(4):
            kv_cp(i, j).wait()

        def branch(br):
            q = jnp.dot(x_buf[br, b], wq_buf[ws, br], preferred_element_type=jnp.float32).astype(jnp.bfloat16)
            os_ = []
            for h in range(hg):
                s = jax.lax.dot_general(q[:, h * dh:(h + 1) * dh], kv_buf[slot, 2 * br, h],
                                        (((1,), (1,)), ((), ())), preferred_element_type=jnp.float32)
                m = jnp.max(s, axis=-1, keepdims=True)
                p = jnp.exp2((s - m) * c)
                l = jnp.sum(p, axis=-1, keepdims=True)
                o = jnp.dot(p.astype(jnp.bfloat16), kv_buf[slot, 2 * br + 1, h],
                            preferred_element_type=jnp.float32)
                os_.append((o * (1.0 / l)).astype(jnp.bfloat16))
            o = jnp.concatenate(os_, axis=-1) if hg > 1 else os_[0]
            return jnp.dot(o, wo_buf[ws, br], preferred_element_type=jnp.float32)

        r = jnp.concatenate([branch(0), branch(1)], axis=-1)

        @pl.when(g == 0)
        def _():
            acc_ref[b] = r

        @pl.when(jnp.logical_and(g > 0, g < ng - 1))
        def _():
            acc_ref[b] += r

        @pl.when(g == ng - 1)
        def _():
            out_buf[b] = (acc_ref[b] + r).astype(out_buf.dtype)
            o_cp(b).start()

    jax.lax.fori_loop(0, nsteps, step, None)
    for b in range(nb):
        o_cp(b).wait()


@jax.jit
def pallas_concat_heads__mha_block_cached__gqa_block_cached__near_ridge_kernel(
    A_x, A_k_cache, A_v_cache, A_wq, A_wo, B_x, B_k_cache, B_v_cache, B_wq, B_wo,
):
    B, Sq, D = A_x.shape
    _, H, Sk, Dh = A_k_cache.shape
    hg, nbuf = HG, NBUF
    bf = A_x.dtype
    return pl.pallas_call(
        functools.partial(_kernel, hg=hg, nbuf=nbuf),
        in_specs=[pl.BlockSpec(memory_space=pl.ANY)] * 10,
        out_specs=pl.BlockSpec(memory_space=pl.ANY),
        out_shape=jax.ShapeDtypeStruct((B, Sq, 2 * D), bf),
        scratch_shapes=[
            pltpu.VMEM((2, B, Sq, D), bf),
            pltpu.VMEM((nbuf, 4, hg, Sk, Dh), bf),
            pltpu.VMEM((2, 2, D, hg * Dh), bf),
            pltpu.VMEM((2, 2, hg * Dh, D), bf),
            pltpu.VMEM((B, Sq, 2 * D), jnp.float32),
            pltpu.VMEM((B, Sq, 2 * D), bf),
            pltpu.SemaphoreType.DMA((2,)),
            pltpu.SemaphoreType.DMA((nbuf, 4)),
            pltpu.SemaphoreType.DMA((2, 4)),
            pltpu.SemaphoreType.DMA((B,)),
        ],
        compiler_params=pltpu.CompilerParams(vmem_limit_bytes=100 * 1024 * 1024),
    )(A_x, A_k_cache, A_v_cache, A_wq, A_wo, B_x, B_k_cache, B_v_cache, B_wq, B_wo)
```

```python
import functools

import jax
import jax.numpy as jnp
import jax.experimental.pallas as pl
import jax.experimental.pallas.tpu as pltpu

HG = 2
NBUF = 4
LOG2E = 1.4426950408889634


def _kernel(ax, ak, av, awq, awo, bx, bk, bv, bwq, bwo, out_hbm,
            x_buf, kv_buf, wq_buf, wo_buf, acc_ref, out_buf,
            x_sem, kv_sem, w_sem, o_sem, *, hg, nbuf):
    nb, sq, d = ax.shape
    nh, dh = ak.shape[1], ak.shape[3]
    ng = nh // hg
    nsteps = ng * nb
    w = hg * dh
    c = (dh ** -0.5) * LOG2E
    kv_src = (ak, av, bk, bv)

    def x_cp(j):
        return pltpu.make_async_copy((ax, bx)[j], x_buf.at[j], x_sem.at[j])

    def kv_cp(i, j):
        slot = i % nbuf
        return pltpu.make_async_copy(
            kv_src[j].at[i % nb, pl.ds((i // nb) * hg, hg)], kv_buf.at[slot, j], kv_sem.at[slot, j])

    def w_cps(g):
        slot = g % 2
        off = g * w if isinstance(g, int) else pl.multiple_of(g * w, w)
        return [
            pltpu.make_async_copy(awq.at[:, pl.ds(off, w)], wq_buf.at[slot, 0], w_sem.at[slot, 0]),
            pltpu.make_async_copy(bwq.at[:, pl.ds(off, w)], wq_buf.at[slot, 1], w_sem.at[slot, 1]),
            pltpu.make_async_copy(awo.at[pl.ds(off, w), :], wo_buf.at[slot, 0], w_sem.at[slot, 2]),
            pltpu.make_async_copy(bwo.at[pl.ds(off, w), :], wo_buf.at[slot, 1], w_sem.at[slot, 3]),
        ]

    def o_cp(b):
        return pltpu.make_async_copy(out_buf.at[b], out_hbm.at[b], o_sem.at[b])

    x_cp(0).start()
    x_cp(1).start()
    for cp in w_cps(0):
        cp.start()
    for i in range(nbuf - 1):
        for j in range(4):
            kv_cp(i, j).start()
    x_cp(0).wait()
    x_cp(1).wait()

    def step(i, _):
        g = i // nb
        b = i % nb
        slot = i % nbuf
        ws = g % 2

        @pl.when(i + nbuf - 1 < nsteps)
        def _():
            for j in range(4):
                kv_cp(i + nbuf - 1, j).start()

        @pl.when(b == 0)
        def _():
            for cp in w_cps(g):
                cp.wait()

            @pl.when(g + 1 < ng)
            def _():
                for cp in w_cps(g + 1):
                    cp.start()

        for j in range(4):
            kv_cp(i, j).wait()

        def branch(br):
            q = jnp.dot(x_buf[br, b], wq_buf[ws, br], preferred_element_type=jnp.float32).astype(jnp.bfloat16)
            os_ = []
            for h in range(hg):
                s = jax.lax.dot_general(q[:, h * dh:(h + 1) * dh], kv_buf[slot, 2 * br, h],
                                        (((1,), (1,)), ((), ())), preferred_element_type=jnp.float32)
                m = jnp.max(s, axis=-1, keepdims=True)
                p = jnp.exp2((s - m) * c)
                l = jnp.sum(p, axis=-1, keepdims=True)
                o = jnp.dot(p.astype(jnp.bfloat16), kv_buf[slot, 2 * br + 1, h],
                            preferred_element_type=jnp.float32)
                os_.append((o * (1.0 / l)).astype(jnp.bfloat16))
            o = jnp.concatenate(os_, axis=-1) if hg > 1 else os_[0]
            return jnp.dot(o, wo_buf[ws, br], preferred_element_type=jnp.float32)

        r = jnp.concatenate([branch(0), branch(1)], axis=-1)

        @pl.when(g == 0)
        def _():
            acc_ref[b] = r

        @pl.when(jnp.logical_and(g > 0, g < ng - 1))
        def _():
            acc_ref[b] += r

        @pl.when(g == ng - 1)
        def _():
            out_buf[b] = (acc_ref[b] + r).astype(out_buf.dtype)
            o_cp(b).start()

    jax.lax.fori_loop(0, nsteps, step, None)
    for b in range(nb):
        o_cp(b).wait()


@jax.jit
def pallas_concat_heads__mha_block_cached__gqa_block_cached__near_ridge_kernel(
    A_x, A_k_cache, A_v_cache, A_wq, A_wo, B_x, B_k_cache, B_v_cache, B_wq, B_wo,
):
    B, Sq, D = A_x.shape
    _, H, Sk, Dh = A_k_cache.shape
    assert A_v_cache.shape == B_k_cache.shape == B_v_cache.shape == A_k_cache.shape
    assert B_x.shape == A_x.shape
    assert A_wq.shape == B_wq.shape == (D, H * Dh)
    assert A_wo.shape == B_wo.shape == (H * Dh, D)
    hg, nbuf = HG, NBUF
    assert H % hg == 0 and (H // hg) * B >= nbuf
    bf = A_x.dtype
    return pl.pallas_call(
        functools.partial(_kernel, hg=hg, nbuf=nbuf),
        in_specs=[pl.BlockSpec(memory_space=pl.ANY)] * 10,
        out_specs=pl.BlockSpec(memory_space=pl.ANY),
        out_shape=jax.ShapeDtypeStruct((B, Sq, 2 * D), bf),
        scratch_shapes=[
            pltpu.VMEM((2, B, Sq, D), bf),
            pltpu.VMEM((nbuf, 4, hg, Sk, Dh), bf),
            pltpu.VMEM((2, 2, D, hg * Dh), bf),
            pltpu.VMEM((2, 2, hg * Dh, D), bf),
            pltpu.VMEM((B, Sq, 2 * D), jnp.float32),
            pltpu.VMEM((B, Sq, 2 * D), bf),
            pltpu.SemaphoreType.DMA((2,)),
            pltpu.SemaphoreType.DMA((nbuf, 4)),
            pltpu.SemaphoreType.DMA((2, 4)),
            pltpu.SemaphoreType.DMA((B,)),
        ],
        compiler_params=pltpu.CompilerParams(vmem_limit_bytes=100 * 1024 * 1024),
    )(A_x, A_k_cache, A_v_cache, A_wq, A_wo, B_x, B_k_cache, B_v_cache, B_wq, B_wo)
```
